```python
import os as _os
_os.environ.setdefault("JAX_PLATFORMS", "cpu")
import jax
import jax.numpy as jnp

def _softmax(x, axis=-1):
    return jax.nn.softmax(x, axis=axis)
def _gelu(x):
    return jax.nn.gelu(x, approximate=True)
def _silu(x):
    return jax.nn.silu(x)
def _sigmoid(x):
    return jax.nn.sigmoid(x)
def _layernorm(x, axis=-1, eps=1e-5):
    m = jnp.mean(x, axis=axis, keepdims=True)
    v = jnp.var(x, axis=axis, keepdims=True)
    return (x - m) / jnp.sqrt(v + eps)
def _scatter_add(tgt, idx, src, axis=0):
    return tgt.at[idx].add(src)
def _segment_sum(src, seg, n):
    return jax.ops.segment_sum(src, seg, n)
class _Rng:
    def __init__(self, key):
        self._k = key
    def _next(self):
        self._k, sub = jax.random.split(self._k)
        return sub
    def normal(self, shape):
        return jax.random.normal(self._next(), shape, dtype=jnp.bfloat16)
    def randint(self, lo, hi, shape):
        return jax.random.randint(self._next(), shape, lo, hi, dtype=jnp.int32)
    def uniform(self, shape, lo=0.0, hi=1.0):
        return jax.random.uniform(self._next(), shape, jnp.bfloat16, lo, hi)
    def permutation(self, n):
        return jax.random.permutation(self._next(), n)


kernel_name = 'gated_mix__mha_block__softmax_full_mha__prompt'

def setup_inputs():
    _rng = _Rng(jax.random.key(int.from_bytes(__import__("os").urandom(4), "little")))
    _w = (lambda a: (lambda t: t.astype(jnp.bfloat16) if jnp.issubdtype(t.dtype, jnp.floating) else t)(jnp.asarray(a)))
    def _A_setup():
        B, S, D, H = 1, 2048, 448, 16
        return {
            "x": _w((lambda *s: _rng.normal(s) * 0.05)(B, S, D)),
            "wqkv": _w((lambda *s: _rng.normal(s) * 0.4)(D, 3 * D)),
            "wo": _w((lambda *s: _rng.normal(s) * 0.05)(D, D)),
        }
    _A_in = _A_setup()

    def _B_setup():
        B, S, D = 1, 2048, 448
        return {
            "x": _w((lambda *s: _rng.normal(s) * 0.05)(B, S, D)),
            "wqkv": _w((lambda *s: _rng.normal(s) * 0.4)(D, 3 * D)),
            "wo": _w((lambda *s: _rng.normal(s) * 0.05)(D, D)),
        }
    _B_in = _B_setup()

    return {
        "A_x": _A_in["x"],
        "A_wqkv": _A_in["wqkv"],
        "A_wo": _A_in["wo"],
        "B_x": _B_in["x"],
        "B_wqkv": _B_in["wqkv"],
        "B_wo": _B_in["wo"],
        "gate_w": _w((lambda *s: _rng.normal(s) * 0.05)(448) * 16.0),
    }

def reference(A_x, A_wqkv, A_wo, B_x, B_wqkv, B_wo, gate_w):
    def _A_ref(x, wqkv, wo):
        B, S, D = x.shape
        H = 16
        Dh = D // H
        qkv = (lambda x, *d: x.transpose(*d))((x @ wqkv).reshape(B, S, 3, H, Dh), 2, 0, 3, 1, 4)
        q, k, v = qkv[0], qkv[1], qkv[2]
        scores = jnp.einsum("bhqd,bhkd->bhqk", q, k) * (Dh ** -0.5)
        p = _softmax(scores, axis=-1)
        o = jnp.einsum("bhqk,bhkd->bhqd", p, v)
        return (lambda x, *d: x.transpose(*d))(o, 0, 2, 1, 3).reshape(B, S, D) @ wo

    def _B_ref(x, wqkv, wo):
        B, S, D = x.shape
        H = 16; Dh = D // H
        qkv = (lambda x, *d: x.transpose(*d))((x @ wqkv).reshape(B, S, 3, H, Dh), 2, 0, 3, 1, 4)
        q, k, v = qkv[0], qkv[1], qkv[2]
        scale = Dh ** -0.5
        scores = jnp.einsum("bhqd,bhkd->bhqk", q, k) * scale
        p = _softmax(scores, axis=-1)
        o = jnp.einsum("bhqk,bhkd->bhqd", p, v)
        return (lambda x, *d: x.transpose(*d))(o, 0, 2, 1, 3).reshape(B, S, D) @ wo

    x = A_x
    g = _sigmoid((x * gate_w).sum(-1, keepdims=True))
    a = _A_ref(x, A_wqkv, A_wo)
    b = _B_ref(x, B_wqkv, B_wo)
    return g * a + (1 - g) * b
```

```python
import jax
import jax.numpy as jnp
import numpy as np
from jax import lax
import jax.experimental.pallas as pl
import jax.experimental.pallas.tpu as pltpu

F32 = jnp.float32
BF16 = jnp.bfloat16
_NN = (((1,), (0,)), ((), ()))
_NT = (((1,), (1,)), ((), ()))

S = 2048
D = 448
H = 16
DH = D // H
SLOT = 32
DS = H * SLOT
BQ = 512
NQ = S // BQ
CK = 128
LOG2E = float(np.log2(np.e))
Q_SCALE = float(DH ** -0.5) * LOG2E
SLAB_OFF = (0, 4 * DH, 8 * DH, D - 128)


def _dot(a, b, dims):
    return lax.dot_general(a, b, dims, preferred_element_type=F32)


def _slot_rows(w):
    z = jnp.zeros((SLOT - DH, w.shape[1]), w.dtype)
    parts = []
    for h in range(H):
        parts += [w[DH * h:DH * (h + 1)], z]
    return jnp.concatenate(parts, axis=0)


def _kernel(xa_hbm, wa_hbm, woa_hbm, wb_hbm, wob_hbm, g_hbm, out_hbm,
            x_v, w_v, wo_v, g_v, wqk_s, wvt_s, wot_s,
            k_s, qt_s, vt_s, gate_s, ot_s, s0, s1, m_s, out_v, in_sem, out_sem):
    cp_wa = pltpu.make_async_copy(wa_hbm, w_v.at[0], in_sem.at[0])
    cp_g = pltpu.make_async_copy(g_hbm, g_v, in_sem.at[1])
    cp_xa = [
        pltpu.make_async_copy(xa_hbm.at[:, pl.ds(c * BQ, BQ)],
                              x_v.at[:, pl.ds(c * BQ, BQ)], in_sem.at[2 + c])
        for c in range(NQ)
    ]
    cp_wb = pltpu.make_async_copy(wb_hbm, w_v.at[1], in_sem.at[6])
    cp_woa = pltpu.make_async_copy(woa_hbm, wo_v.at[0], in_sem.at[7])
    cp_wob = pltpu.make_async_copy(wob_hbm, wo_v.at[1], in_sem.at[8])
    cp_wa.start()
    cp_g.start()
    for cp in cp_xa:
        cp.start()

    def prep_weights(b):
        wqk_s[b, 0:D, :] = w_v[b, :, 0:D].T
        wqk_s[b, D:2 * D, :] = w_v[b, :, D:2 * D].T
        wvt_s[b] = _slot_rows(w_v[b, :, 2 * D:3 * D].T)

    def project(b, c):
        ones_row = lax.broadcasted_iota(jnp.int32, (DS, BQ), 0) % SLOT == DH
        ts = pl.ds(c * BQ, BQ)
        xt = x_v[:, ts]
        qt = _dot(wqk_s[b, 0:D, :], xt, _NN)
        qt_s[b, :, ts] = (qt * Q_SCALE).astype(BF16)
        if b == 0:
            kt = _dot(wqk_s[0, D:2 * D + 16, :], xt, _NN)
            g = jax.nn.sigmoid(kt[D:D + 8])
            gate_s[0, :, ts] = jnp.broadcast_to(g[0:1], (8, BQ))
            gate_s[1, :, ts] = jnp.broadcast_to(1.0 - g[0:1], (8, BQ))
        else:
            kt = _dot(wqk_s[1, D:2 * D, :], xt, _NN)
        kt = kt[0:D].astype(BF16)
        for j, off in enumerate(SLAB_OFF):
            k_s[b * 4 + j, ts, :] = kt[off:off + 128].T
        vt = _dot(wvt_s[b], xt, _NN)
        vt_s[pl.ds(b * DS, DS), ts] = jnp.where(ones_row, 1.0, vt).astype(BF16)

    cp_wa.wait()
    cp_wb.start()
    cp_woa.start()
    cp_wob.start()
    prep_weights(0)
    cp_g.wait()
    grow = jnp.broadcast_to(g_v[...].astype(F32), (16, D))
    first = lax.broadcasted_iota(jnp.int32, (16, D), 0) == 0
    wqk_s[0, 2 * D:2 * D + 16, :] = jnp.where(first, grow, 0.0).astype(BF16)
    for c in range(NQ):
        cp_xa[c].wait()
        if c == 2:
            cp_wb.wait()
            cp_woa.wait()
            cp_wob.wait()
            prep_weights(1)
            for b in range(2):
                wot_s[:, b * DS:(b + 1) * DS] = _slot_rows(wo_v[b]).T
        project(0, c)
    for c in range(NQ):
        project(1, c)

    def step(cur, nxt, s_cur, s_nxt, tail=None):
        if nxt is not None:
            nb, nj, nh = nxt // H, (nxt % H) // 4, nxt % 4
            r0 = jnp.where(nj == 3, SLAB_OFF[3], nj * (4 * DH))
            lo = (nh * DH + jnp.where(nj == 3, 16, 0)) // 2
            word = lax.broadcasted_iota(jnp.int32, (64, BQ), 0)
            keep = (word >= lo) & (word < lo + DH // 2)
        for q in range(NQ):
            qs = pl.ds(q * BQ, BQ)
            if nxt is not None:
                qm = qt_s[nb, pl.ds(pl.multiple_of(r0, 16), 128), qs]
                qm = pltpu.bitcast(qm, jnp.uint32)
                qm = pltpu.bitcast(jnp.where(keep, qm, jnp.uint32(0)), BF16)
            if cur is not None:
                m = m_s[:, qs]
                row = pl.multiple_of(cur * SLOT, SLOT)
            mn = acc = None
            for c in range(S // CK):
                ks = pl.ds(c * CK, CK)
                if nxt is not None:
                    st = _dot(k_s[nb * 4 + nj, ks, :], qm, _NN)
                    s_nxt[ks, qs] = st
                    cm = jnp.max(st.reshape(CK // 8, 8, BQ), axis=0)
                    mn = cm if mn is None else jnp.maximum(mn, cm)
                if cur is not None:
                    p = jnp.exp2(s_cur[ks, qs] - m).astype(BF16)
                    a = _dot(vt_s[pl.ds(row, SLOT), ks], p, _NN)
                    acc = a if acc is None else acc + a
            if cur is not None:
                scale = gate_s[cur // H, 0:1, qs] / acc[DH:DH + 1]
                ot_s[pl.ds(row, SLOT), qs] = (acc * scale).astype(BF16)
            if nxt is not None:
                m_s[:, qs] = jnp.max(mn, axis=0, keepdims=True)
            if tail is not None:
                tail(q)

    step(None, jnp.int32(0), None, s0)

    def body(i, carry):
        @pl.when(i % 2 == 0)
        def _():
            step(i, i + 1, s0, s1)

        @pl.when(i % 2 == 1)
        def _():
            step(i, i + 1, s1, s0)
        return carry

    lax.fori_loop(0, 2 * H - 1, body, 0)

    def out_copy(q):
        cols = pl.ds(q * BQ, BQ)
        return pltpu.make_async_copy(out_v.at[:, cols], out_hbm.at[:, cols], out_sem.at[q])

    def out_proj(q):
        if q > 0:
            qs = pl.ds((q - 1) * BQ, BQ)
            out_v[:, qs] = _dot(wot_s[...], ot_s[:, qs], _NN).astype(BF16)
            if q > 1:
                out_copy(q - 2).start()

    step(jnp.int32(2 * H - 1), None, s1, None, tail=out_proj)
    qs = pl.ds((NQ - 1) * BQ, BQ)
    out_copy(NQ - 2).start()
    out_v[:, qs] = _dot(wot_s[...], ot_s[:, qs], _NN).astype(BF16)
    out_copy(NQ - 1).start()
    for q in range(NQ):
        out_copy(q).wait()


@jax.jit
def pallas_gated_mix__mha_block__softmax_full_mha__prompt_kernel(
    A_x: jax.Array,
    A_wqkv: jax.Array,
    A_wo: jax.Array,
    B_x: jax.Array,
    B_wqkv: jax.Array,
    B_wo: jax.Array,
    gate_w: jax.Array,
):
    del B_x
    hbm = pl.BlockSpec(memory_space=pltpu.MemorySpace.HBM)
    out_t = pl.pallas_call(
        _kernel,
        out_shape=jax.ShapeDtypeStruct((D, S), BF16),
        in_specs=[hbm] * 6,
        out_specs=hbm,
        scratch_shapes=[
            pltpu.VMEM((D, S), BF16),
            pltpu.VMEM((2, D, 3 * D), BF16),
            pltpu.VMEM((2, D, D), BF16),
            pltpu.VMEM((1, D), BF16),
            pltpu.VMEM((2, 2 * D + 16, D), BF16),
            pltpu.VMEM((2, DS, D), BF16),
            pltpu.VMEM((D, 2 * DS), BF16),
            pltpu.VMEM((8, S, 128), BF16),
            pltpu.VMEM((2, D, S), BF16),
            pltpu.VMEM((2 * DS, S), BF16),
            pltpu.VMEM((2, 8, S), F32),
            pltpu.VMEM((2 * DS, S), BF16),
            pltpu.VMEM((S, S), F32),
            pltpu.VMEM((S, S), F32),
            pltpu.VMEM((1, S), F32),
            pltpu.VMEM((D, S), BF16),
            pltpu.SemaphoreType.DMA((9,)),
            pltpu.SemaphoreType.DMA((NQ,)),
        ],
        compiler_params=pltpu.CompilerParams(vmem_limit_bytes=100 * 1024 * 1024),
    )(A_x[0].T, A_wqkv, A_wo, B_wqkv, B_wo, gate_w.reshape(1, D))
    return out_t.T[None]
```

```python
import jax
import jax.numpy as jnp
import numpy as np
from jax import lax
import jax.experimental.pallas as pl
import jax.experimental.pallas.tpu as pltpu

F32 = jnp.float32
BF16 = jnp.bfloat16
_NN = (((1,), (0,)), ((), ()))
_NT = (((1,), (1,)), ((), ()))

S = 2048
D = 448
H = 16
DH = D // H
SLOT = 32
DS = H * SLOT
BQ = 512
NQ = S // BQ
G = 2
CK = 128
LOG2E = float(np.log2(np.e))
Q_SCALE = float(DH ** -0.5) * LOG2E
SLAB_OFF = (0, 4 * DH, 8 * DH, D - 128)


def _dot(a, b, dims):
    return lax.dot_general(a, b, dims, preferred_element_type=F32)


def _slot_v(vt):
    n = vt.shape[1]
    pad = (lax.broadcasted_iota(jnp.int32, (SLOT - DH, n), 0) == 0).astype(vt.dtype)
    parts = []
    for h in range(H):
        parts += [vt[DH * h:DH * (h + 1)], pad]
    return jnp.concatenate(parts, axis=0)


def _unslot(ot):
    return jnp.concatenate(
        [ot[SLOT * h:SLOT * h + DH] for h in range(ot.shape[0] // SLOT)], axis=0)


def _kernel(x_hbm, wa_hbm, woa_hbm, wb_hbm, wob_hbm, g_hbm, out_hbm,
            x_v, w_v, wo_v, g_v, wt_s, wot_s,
            k_s, qt_s, vt_s, gate_s, ot_s, oc_s, part_s, out_v, in_sem, out_sem, *sm_refs):
    s_refs, m_refs = sm_refs[0:G], sm_refs[G:2 * G]
    cp_wa = [
        pltpu.make_async_copy(wa_hbm.at[:, lo:hi], w_v.at[0, :, lo:hi], in_sem.at[7 + i])
        for i, (lo, hi) in enumerate(((2 * D, 3 * D), (384, 2 * D), (0, 384)))
    ]
    cp_g = pltpu.make_async_copy(g_hbm, g_v, in_sem.at[1])
    cp_x0 = pltpu.make_async_copy(x_hbm.at[:, 0:BQ], x_v.at[:, 0:BQ], in_sem.at[2])
    cp_x1 = pltpu.make_async_copy(x_hbm.at[:, BQ:S], x_v.at[:, BQ:S], in_sem.at[3])
    cp_wb = pltpu.make_async_copy(wb_hbm, w_v.at[1], in_sem.at[4])
    cp_woa = pltpu.make_async_copy(woa_hbm, wo_v.at[0], in_sem.at[5])
    cp_wob = pltpu.make_async_copy(wob_hbm, wo_v.at[1], in_sem.at[6])
    cp_wa[0].start()
    cp_x0.start()
    cp_g.start()
    cp_wa[1].start()
    cp_wa[2].start()

    def prep_v(b):
        wt_s[b, 2 * D + 16:3 * D + 16, :] = w_v[b, :, 2 * D:3 * D].T

    def prep_k(b):
        wt_s[b, D:2 * D, :] = w_v[b, :, D:2 * D].T
        wt_s[b, 2 * D:2 * D + 16, :] = gate_tile()

    def prep_q(b):
        wt_s[b, 0:D, :] = w_v[b, :, 0:D].T

    def project(b, c, hooks=(None, None, None)):
        ts = pl.ds(pl.multiple_of(c * BQ, BQ), BQ)
        if hooks[0] is not None:
            hooks[0]()
        xt = x_v[:, ts]
        vt = _dot(wt_s[b, 2 * D + 16:3 * D + 16, :], xt, _NN)
        vt_s[pl.ds(pl.multiple_of(b * DS, DS), DS), ts] = _slot_v(vt).astype(BF16)
        if hooks[1] is not None:
            hooks[1]()
        kt = _dot(wt_s[b, D:2 * D + 16, :], xt, _NN)
        g = jax.nn.sigmoid(kt[D:D + 8])[0:1]
        gate_s[b, 0, :, ts] = jnp.broadcast_to(g, (8, BQ))
        gate_s[b, 1, :, ts] = jnp.broadcast_to(1.0 - g, (8, BQ))
        kt = kt[0:D].astype(BF16)
        for j, off in enumerate(SLAB_OFF):
            k_s[b * 4 + j, ts, :] = kt[off:off + 128].T
        if hooks[2] is not None:
            hooks[2]()
        qt = _dot(wt_s[b, 0:D, :], xt, _NN)
        qt_s[b, :, ts] = (qt * Q_SCALE).astype(BF16)

    def hook0():
        cp_wa[0].wait()
        prep_v(0)
        cp_x0.wait()
        cp_g.wait()
        cp_wb.start()
        cp_x1.start()
        cp_woa.start()
        cp_wob.start()

    def hook1():
        cp_wa[1].wait()
        cp_wa[2].wait()
        prep_k(0)
        prep_q(0)

    def hook2():
        cp_wb.wait()
        prep_v(1)
        prep_k(1)
        prep_q(1)

    def gate_tile():
        grow = jnp.broadcast_to(g_v[...].astype(F32).reshape(1, D), (16, D))
        first = lax.broadcasted_iota(jnp.int32, (16, D), 0) == 0
        return jnp.where(first, grow, 0.0).astype(BF16)

    project(0, 0, (hook0, hook1, hook2))
    cp_x1.wait()

    def proj_body(i, carry):
        project(i // NQ, i % NQ)
        return carry

    lax.fori_loop(1, 2 * NQ, proj_body, 0)

    def step(cur, nxt, s_ref, m_s, qs_list=None, hook=None):
        if nxt is not None:
            nb, nj, nh = nxt // H, (nxt % H) // 4, nxt % 4
            r0 = jnp.where(nj == 3, SLAB_OFF[3], nj * (4 * DH))
            lo = (nh * DH + jnp.where(nj == 3, 16, 0)) // 2
            word = lax.broadcasted_iota(jnp.int32, (64, BQ), 0)
            keep = (word >= lo) & (word < lo + DH // 2)
        for q, qs in [(q, pl.ds(q * BQ, BQ)) for q in range(NQ)] if qs_list is None else qs_list:
            if nxt is not None:
                qm = qt_s[nb, pl.ds(pl.multiple_of(r0, 16), 128), qs]
                qm = pltpu.bitcast(qm, jnp.uint32)
                qm = pltpu.bitcast(jnp.where(keep, qm, jnp.uint32(0)), BF16)
            if cur is not None:
                m = m_s[:, qs]
                row = pl.multiple_of(cur * SLOT, SLOT)
            mn = acc = None
            for c in range(S // CK):
                ks = pl.ds(c * CK, CK)
                if cur is not None:
                    p = jnp.exp2(s_ref[q, ks, :] - m).astype(BF16)
                    a = _dot(vt_s[pl.ds(row, SLOT), ks], p, _NN)
                    acc = a if acc is None else acc + a
                if nxt is not None:
                    st = _dot(k_s[nb * 4 + nj, ks, :], qm, _NN)
                    s_ref[q, ks, :] = st
                    cm = jnp.max(st.reshape(CK // 8, 8, BQ), axis=0)
                    mn = cm if mn is None else jnp.maximum(mn, cm)
                if hook is not None:
                    hook(c)
            if cur is not None:
                scale = gate_s[0, cur // H, 0:1, qs] / acc[DH:DH + 1]
                ot_s[pl.ds(row, SLOT), qs] = (acc * scale).astype(BF16)
            if nxt is not None:
                m_s[:, qs] = jnp.max(mn, axis=0, keepdims=True)

    def wo_prep(c):
        if c in (1, 2):
            b = c - 1
            wot_s[:, b * D:(b + 1) * D] = wo_v[b].T

    cp_woa.wait()
    cp_wob.wait()
    for g in range(G):
        step(None, jnp.int32(g), s_refs[g], m_refs[g],
             qs_list=[(0, pl.ds(0, BQ))] if g == 0 else [], hook=wo_prep if g == 0 else None)
        step(None, jnp.int32(g), s_refs[g], m_refs[g],
             qs_list=[(q, pl.ds(q * BQ, BQ)) for q in range(0 if g else 1, NQ)])

    def body(i, carry):
        for g in range(G):
            step(i * G + g, i * G + g + G, s_refs[g], m_refs[g])
        return carry

    lax.fori_loop(0, 2 * H // G - 1, body, 0)

    def cols(q):
        return pl.ds(pl.multiple_of(q * BQ, BQ), BQ)

    def out_copy(q):
        return pltpu.make_async_copy(out_v.at[:, cols(q)], out_hbm.at[:, cols(q)], out_sem.at[q])

    KP = 768
    hp = -(-KP // DH)
    h0 = KP // DH
    RG = 64
    n_hook = G * (S // CK)
    at = [(i + 1) * n_hook * RG // D - 1 for i in range(D // RG)]

    def partial_proj(q):
        oc_s[0:KP, :] = _unslot(ot_s[0:hp * SLOT, cols(q)])[0:KP]

        def piece(c):
            if c in at:
                rows = pl.ds(at.index(c) * RG, RG)
                part_s[rows, :] = _dot(wot_s[rows, 0:KP], oc_s[0:KP, :], _NN)
        return piece

    def final_proj(q):
        tail = _unslot(ot_s[h0 * SLOT:2 * H * SLOT, cols(q)])[KP - h0 * DH:]
        out = part_s[...] + _dot(wot_s[:, KP:2 * D], tail, _NN)
        out_v[:, cols(q)] = out.astype(BF16)

    def last_heads(q):
        hook = partial_proj(q)
        for g in range(G):
            step(jnp.int32(2 * H - G + g), None, s_refs[g], m_refs[g], [(q, cols(q))],
                 hook=lambda c, g=g: hook(g * (S // CK) + c))

    last_heads(0)

    def tail_body(q, carry):
        final_proj(q - 1)
        last_heads(q)
        out_copy(q - 1).start()
        return carry

    lax.fori_loop(1, NQ, tail_body, 0)
    final_proj(NQ - 1)
    out_copy(NQ - 1).start()
    for q in range(NQ):
        out_copy(q).wait()


@jax.jit
def pallas_gated_mix__mha_block__softmax_full_mha__prompt_kernel(
    A_x: jax.Array,
    A_wqkv: jax.Array,
    A_wo: jax.Array,
    B_x: jax.Array,
    B_wqkv: jax.Array,
    B_wo: jax.Array,
    gate_w: jax.Array,
):
    del B_x
    hbm = pl.BlockSpec(memory_space=pltpu.MemorySpace.HBM)
    out_t = pl.pallas_call(
        _kernel,
        out_shape=jax.ShapeDtypeStruct((D, S), BF16),
        in_specs=[hbm] * 6,
        out_specs=hbm,
        scratch_shapes=[
            pltpu.VMEM((D, S), BF16),
            pltpu.VMEM((2, D, 3 * D), BF16),
            pltpu.VMEM((2, D, D), BF16),
            pltpu.VMEM((D,), BF16),
            pltpu.VMEM((2, 3 * D + 16, D), BF16),
            pltpu.VMEM((D, 2 * D), BF16),
            pltpu.VMEM((8, S, 128), BF16),
            pltpu.VMEM((2, D, S), BF16),
            pltpu.VMEM((2 * DS, S), BF16),
            pltpu.VMEM((2, 2, 8, S), F32),
            pltpu.VMEM((2 * DS, S), BF16),
            pltpu.VMEM((768, BQ), BF16),
            pltpu.VMEM((D, BQ), F32),
            pltpu.VMEM((D, S), BF16),
            pltpu.SemaphoreType.DMA((10,)),
            pltpu.SemaphoreType.DMA((NQ,)),
        ] + [pltpu.VMEM((NQ, S, BQ), F32)] * G + [
            pltpu.VMEM((1, S), F32)] * G,
        compiler_params=pltpu.CompilerParams(vmem_limit_bytes=120 * 1024 * 1024),
    )(A_x[0].T, A_wqkv, A_wo, B_wqkv, B_wo, gate_w)
    return out_t.T[None]
```

```python
import jax
import jax.numpy as jnp
import numpy as np
from jax import lax
import jax.experimental.pallas as pl
import jax.experimental.pallas.tpu as pltpu

F32 = jnp.float32
BF16 = jnp.bfloat16
U32 = jnp.uint32
_NN = (((1,), (0,)), ((), ()))

S = 2048
D = 448
H = 16
DH = D // H
SLOT = 32
DS = H * SLOT
HD = D // 2
BQ = 512
NQ = S // BQ
G = 2
CK = 256
LOG2E = float(np.log2(np.e))
Q_SCALE = float(DH ** -0.5) * LOG2E
SLAB_OFF = (0, 4 * DH, 8 * DH, D - 128)


def _dot(a, b, dims):
    return lax.dot_general(a, b, dims, preferred_element_type=F32)


def _words(x):
    return pltpu.bitcast(x.astype(BF16), jnp.uint32)


def _halves(x):
    return pltpu.bitcast(x, BF16)


def _slot_v(vt):
    n = vt.shape[1]
    pad = (lax.broadcasted_iota(jnp.int32, (SLOT - DH, n), 0) == 0).astype(vt.dtype)
    parts = []
    for h in range(H):
        parts += [vt[DH * h:DH * (h + 1)], pad]
    return jnp.concatenate(parts, axis=0)


def _unslot(ot):
    w = SLOT // 2
    return jnp.concatenate(
        [ot[w * h:w * h + DH // 2] for h in range(ot.shape[0] // w)], axis=0)


def _kernel(x_hbm, wa_hbm, woa_hbm, wb_hbm, wob_hbm, g_hbm, out_hbm,
            x_v, w_v, wo_v, g_v, wt_s, wot_s,
            k_s, qt_s, vt_s, gate_s, ot_s, oc_s, part_s, out_v, in_sem, out_sem, *sm_refs):
    s_refs, m_refs = sm_refs[0:G], sm_refs[G:2 * G]
    cp_wa = [
        pltpu.make_async_copy(wa_hbm.at[:, lo:hi], w_v.at[0, :, lo:hi], in_sem.at[7 + i])
        for i, (lo, hi) in enumerate(((2 * D, 3 * D), (384, 2 * D), (0, 384)))
    ]
    cp_g = pltpu.make_async_copy(g_hbm, g_v, in_sem.at[1])
    cp_x0 = pltpu.make_async_copy(x_hbm.at[:, 0:BQ], x_v.at[:, 0:BQ], in_sem.at[2])
    cp_x1 = pltpu.make_async_copy(x_hbm.at[:, BQ:S], x_v.at[:, BQ:S], in_sem.at[3])
    cp_wb = pltpu.make_async_copy(wb_hbm, w_v.at[1], in_sem.at[4])
    cp_woa = pltpu.make_async_copy(woa_hbm, wo_v.at[0], in_sem.at[5])
    cp_wob = pltpu.make_async_copy(wob_hbm, wo_v.at[1], in_sem.at[6])
    cp_wa[0].start()
    cp_x0.start()
    cp_g.start()
    cp_wa[1].start()
    cp_wa[2].start()

    def prep_v(b):
        wt_s[b, D + 8:3 * HD + 8, :] = _words(w_v[b, :, 2 * D:3 * D].T)

    def prep_k(b):
        wt_s[b, HD:D, :] = _words(w_v[b, :, D:2 * D].T)
        wt_s[b, D:D + 8, :] = _words(gate_tile())

    def prep_q(b):
        wt_s[b, 0:HD, :] = _words(w_v[b, :, 0:D].T)

    def project(b, c, hooks=(None, None, None)):
        ts = pl.ds(pl.multiple_of(c * BQ, BQ), BQ)
        if hooks[0] is not None:
            hooks[0]()
        xt = x_v[:, ts]
        vrows = pl.ds(pl.multiple_of(b * (DS // 2), DS // 2), DS // 2)
        if hooks[1] is None:
            vt = _dot(_halves(wt_s[b, D + 8:3 * HD + 8, :]), xt, _NN)
            vt_s[vrows, ts] = _words(_slot_v(vt))
        else:
            for i in range(2):
                hs = pl.ds(c * BQ + i * (BQ // 2), BQ // 2)
                vt = _dot(_halves(wt_s[b, D + 8:3 * HD + 8, :]), x_v[:, hs], _NN)
                vt_s[vrows, hs] = _words(_slot_v(vt))
                hooks[1](i)
        kt = _dot(_halves(wt_s[b, HD:D + 8, :]), xt, _NN)
        g = jax.nn.sigmoid(kt[D:D + 8])[0:1]
        gate_s[b, 0, :, ts] = jnp.broadcast_to(g, (8, BQ))
        gate_s[b, 1, :, ts] = jnp.broadcast_to(1.0 - g, (8, BQ))
        kt = kt[0:D].astype(BF16)
        for j, off in enumerate(SLAB_OFF):
            k_s[b * 4 + j, pl.ds(pl.multiple_of(c * (BQ // 2), BQ // 2), BQ // 2), :] = (
                _words(kt[off:off + 128].T))
        if hooks[2] is not None:
            hooks[2]()
        qt = _dot(_halves(wt_s[b, 0:HD, :]), xt, _NN)
        qt_s[b, :, ts] = _words(qt * Q_SCALE)

    def hook0():
        cp_wa[0].wait()
        prep_v(0)
        cp_x0.wait()
        cp_g.wait()
        cp_wb.start()
        cp_x1.start()
        cp_woa.start()
        cp_wob.start()

    def hook1(i):
        if i == 0:
            cp_wa[1].wait()
            cp_wa[2].wait()
            prep_k(0)
        else:
            prep_q(0)

    def hook2():
        cp_wb.wait()
        prep_v(1)
        prep_k(1)
        prep_q(1)

    def gate_tile():
        grow = jnp.broadcast_to(g_v[...].astype(F32).reshape(1, D), (16, D))
        first = lax.broadcasted_iota(jnp.int32, (16, D), 0) == 0
        return jnp.where(first, grow, 0.0).astype(BF16)

    project(0, 0, (hook0, hook1, hook2))
    cp_x1.wait()

    def proj_body(i, carry):
        project(i >> 2, i & 3)
        return carry

    lax.fori_loop(1, 2 * NQ, proj_body, 0)

    def step(cur, nxt, s_ref, m_s, qs_list=None, hook=None):
        if nxt is not None:
            nb, nj, nh = nxt >> 4, (nxt >> 2) & 3, nxt & 3
            r0 = jnp.where(nj == 3, SLAB_OFF[3] // 2, nj * (2 * DH))
            lo = nh * (DH // 2) + jnp.where(nj == 3, 8, 0)
            word = lax.broadcasted_iota(jnp.int32, (64, BQ), 0)
            keep = (word >= lo) & (word < lo + DH // 2)
        for q, qs in [(q, pl.ds(q * BQ, BQ)) for q in range(NQ)] if qs_list is None else qs_list:
            if nxt is not None:
                qm = qt_s[nb, pl.ds(pl.multiple_of(r0, 8), 64), qs]
                qm = _halves(jnp.where(keep, qm, jnp.zeros_like(qm)))
            if cur is not None:
                m = m_s[:, qs]
                vrow = pl.multiple_of(cur * (SLOT // 2), SLOT // 2)
            mn = acc = None
            for c in range(S // CK):
                ks = pl.ds(c * CK, CK)
                if cur is not None:
                    p = jnp.exp2(s_ref[q, ks, :] - m).astype(BF16)
                    a = _dot(_halves(vt_s[pl.ds(vrow, SLOT // 2), ks]), p, _NN)
                    acc = a if acc is None else acc + a
                if nxt is not None:
                    st = _dot(_halves(k_s[nb * 4 + nj, pl.ds(c * (CK // 2), CK // 2), :]), qm, _NN)
                    s_ref[q, ks, :] = st
                    cm = jnp.max(st.reshape(CK // 8, 8, BQ), axis=0)
                    mn = cm if mn is None else jnp.maximum(mn, cm)
                if hook is not None:
                    hook(c)
            if cur is not None:
                scale = gate_s[0, cur >> 4, 0:1, qs] * pl.reciprocal(acc[DH:DH + 1], approx=False)
                ot_s[pl.ds(vrow, SLOT // 2), qs] = _words(acc * scale)
            if nxt is not None:
                m_s[:, qs] = jnp.max(mn, axis=0, keepdims=True)

    def wo_prep(c):
        if c in (1, 2):
            b = c - 1
            wot_s[:, b * D:(b + 1) * D] = _words(wo_v[b].T)

    cp_woa.wait()
    cp_wob.wait()
    for g in range(G):
        step(None, jnp.int32(g), s_refs[g], m_refs[g],
             qs_list=[(0, pl.ds(0, BQ))] if g == 0 else [], hook=wo_prep if g == 0 else None)
        step(None, jnp.int32(g), s_refs[g], m_refs[g],
             qs_list=[(q, pl.ds(q * BQ, BQ)) for q in range(0 if g else 1, NQ)])

    def body(i, carry):
        for g in range(G):
            step(i * G + g, i * G + g + G, s_refs[g], m_refs[g])
        return carry

    lax.fori_loop(0, 2 * H // G - 1, body, 0)

    def cols(q):
        return pl.ds(pl.multiple_of(q * BQ, BQ), BQ)

    def out_copy(q):
        return pltpu.make_async_copy(out_v.at[:, cols(q)], out_hbm.at[:, cols(q)], out_sem.at[q])

    KP = 768
    hp = -(-KP // DH)
    h0 = KP // DH
    RG = 64
    n_hook = G * (S // CK)
    at = [(i + 1) * n_hook * RG // D - 1 for i in range(D // RG)]

    def partial_proj(q):
        oc_s[...] = _unslot(ot_s[0:hp * SLOT // 2, cols(q)])[0:KP // 2]

        def piece(c):
            if c in at:
                i = at.index(c)
                w = _halves(wot_s[pl.ds(i * RG // 2, RG // 2), 0:KP])
                part_s[pl.ds(i * RG, RG), :] = _dot(w, _halves(oc_s[...]), _NN)
        return piece

    def final_proj(q):
        tail = _unslot(ot_s[h0 * SLOT // 2:, cols(q)])[(KP - h0 * DH) // 2:]
        out = part_s[...] + _dot(_halves(wot_s[:, KP:2 * D]), _halves(tail), _NN)
        out_v[:, cols(q)] = out.astype(BF16)

    def last_heads(q):
        hook = partial_proj(q)
        for g in range(G):
            step(jnp.int32(2 * H - G + g), None, s_refs[g], m_refs[g], [(q, cols(q))],
                 hook=lambda c, g=g: hook(g * (S // CK) + c))

    last_heads(0)

    def tail_body(q, carry):
        final_proj(q - 1)
        last_heads(q)
        out_copy(q - 1).start()
        return carry

    lax.fori_loop(1, NQ, tail_body, 0)
    final_proj(NQ - 1)
    out_copy(NQ - 1).start()
    for q in range(NQ):
        out_copy(q).wait()


@jax.jit
def pallas_gated_mix__mha_block__softmax_full_mha__prompt_kernel(
    A_x: jax.Array,
    A_wqkv: jax.Array,
    A_wo: jax.Array,
    B_x: jax.Array,
    B_wqkv: jax.Array,
    B_wo: jax.Array,
    gate_w: jax.Array,
):
    del B_x
    hbm = pl.BlockSpec(memory_space=pltpu.MemorySpace.HBM)
    out_t = pl.pallas_call(
        _kernel,
        out_shape=jax.ShapeDtypeStruct((D, S), BF16),
        in_specs=[hbm] * 6,
        out_specs=hbm,
        scratch_shapes=[
            pltpu.VMEM((D, S), BF16),
            pltpu.VMEM((2, D, 3 * D), BF16),
            pltpu.VMEM((2, D, D), BF16),
            pltpu.VMEM((D,), BF16),
            pltpu.VMEM((2, 3 * HD + 8, D), U32),
            pltpu.VMEM((D // 2, 2 * D), U32),
            pltpu.VMEM((8, S // 2, 128), U32),
            pltpu.VMEM((2, D // 2, S), U32),
            pltpu.VMEM((DS, S), U32),
            pltpu.VMEM((2, 2, 8, S), F32),
            pltpu.VMEM((DS, S), U32),
            pltpu.VMEM((384, BQ), U32),
            pltpu.VMEM((D, BQ), F32),
            pltpu.VMEM((D, S), BF16),
            pltpu.SemaphoreType.DMA((10,)),
            pltpu.SemaphoreType.DMA((NQ,)),
        ] + [pltpu.VMEM((NQ, S, BQ), F32)] * G + [
            pltpu.VMEM((1, S), F32)] * G,
        compiler_params=pltpu.CompilerParams(
            vmem_limit_bytes=120 * 1024 * 1024,
            flags={"XLA_TPU_EVENLY_DISTRIBUTE_CRITICAL_NODES": True},
        ),
    )(A_x.reshape(S, D).T, A_wqkv, A_wo, B_wqkv, B_wo, gate_w)
    return out_t.T[None]
```
